```python
import os as _os
_os.environ.setdefault("JAX_PLATFORMS", "cpu")
import jax
import jax.numpy as jnp

def _softmax(x, axis=-1):
    return jax.nn.softmax(x, axis=axis)
def _gelu(x):
    return jax.nn.gelu(x, approximate=True)
def _silu(x):
    return jax.nn.silu(x)
def _sigmoid(x):
    return jax.nn.sigmoid(x)
def _layernorm(x, axis=-1, eps=1e-5):
    m = jnp.mean(x, axis=axis, keepdims=True)
    v = jnp.var(x, axis=axis, keepdims=True)
    return (x - m) / jnp.sqrt(v + eps)
def _scatter_add(tgt, idx, src, axis=0):
    return tgt.at[idx].add(src)
def _segment_sum(src, seg, n):
    return jax.ops.segment_sum(src, seg, n)
class _Rng:
    def __init__(self, key):
        self._k = key
    def _next(self):
        self._k, sub = jax.random.split(self._k)
        return sub
    def normal(self, shape):
        return jax.random.normal(self._next(), shape, dtype=jnp.bfloat16)
    def randint(self, lo, hi, shape):
        return jax.random.randint(self._next(), shape, lo, hi, dtype=jnp.int32)
    def uniform(self, shape, lo=0.0, hi=1.0):
        return jax.random.uniform(self._next(), shape, jnp.bfloat16, lo, hi)
    def permutation(self, n):
        return jax.random.permutation(self._next(), n)


kernel_name = 'interleave_layers__mha_block__dense_activation_mish__prompt'

def setup_inputs():
    _rng = _Rng(jax.random.key(int.from_bytes(__import__("os").urandom(4), "little")))
    _w = (lambda a: (lambda t: t.astype(jnp.bfloat16) if jnp.issubdtype(t.dtype, jnp.floating) else t)(jnp.asarray(a)))
    def _A_setup():
        B, S, D, H = 1, 2048, 512, 32
        return {
            "x": _w((lambda *s: _rng.normal(s) * 0.05)(B, S, D)),
            "wqkv": _w((lambda *s: _rng.normal(s) * 0.05)(D, 3 * D)),
            "wo": _w((lambda *s: _rng.normal(s) * 0.05)(D, D)),
        }
    _A_in = _A_setup()

    def _B_setup():
        B, S, D, F = 1, 2048, 512, 1792
        return {
            "x": _w((lambda *s: _rng.normal(s) * 0.05)(B, S, D)),
            "w1": _w((lambda *s: _rng.normal(s) * 0.4)(D, F) * (D ** -0.5)),
            "b1": _w((lambda *s: _rng.normal(s) * 0.4)(F)),
            "w2": _w((lambda *s: _rng.normal(s) * 0.4)(F, D) * (F ** -0.5)),
        }
    _B_in = _B_setup()

    return {
        "A_x": _A_in["x"],
        "A_wqkv": _A_in["wqkv"],
        "A_wo": _A_in["wo"],
        "B_x": _B_in["x"],
        "B_w1": _B_in["w1"],
        "B_b1": _B_in["b1"],
        "B_w2": _B_in["w2"],
    }

def reference(A_x, A_wqkv, A_wo, B_x, B_w1, B_b1, B_w2):
    def _A_ref(x, wqkv, wo):
        B, S, D = x.shape
        H = 32
        Dh = D // H
        qkv = (lambda x, *d: x.transpose(*d))((x @ wqkv).reshape(B, S, 3, H, Dh), 2, 0, 3, 1, 4)
        q, k, v = qkv[0], qkv[1], qkv[2]
        scores = jnp.einsum("bhqd,bhkd->bhqk", q, k) * (Dh ** -0.5)
        p = _softmax(scores, axis=-1)
        o = jnp.einsum("bhqk,bhkd->bhqd", p, v)
        return (lambda x, *d: x.transpose(*d))(o, 0, 2, 1, 3).reshape(B, S, D) @ wo

    def _B_ref(x, w1, b1, w2):
        h = jnp.einsum("bsd,df->bsf", x, w1) + b1
        sp = jnp.log1p(jnp.exp(-jnp.abs(h))) + jnp.where(h > 0, h, jnp.zeros_like(h))
        act = h * jnp.tanh(sp)
        return jnp.einsum("bsf,fd->bsd", act, w2)

    x = A_x
    x = x + _A_ref(_layernorm(x, axis=-1), A_wqkv, A_wo)
    x = x + _B_ref(_layernorm(x, axis=-1), B_w1, B_b1, B_w2)
    x = x + _A_ref(_layernorm(x, axis=-1), A_wqkv, A_wo)
    x = x + _B_ref(_layernorm(x, axis=-1), B_w1, B_b1, B_w2)
    return x
```

```python
import functools
import jax
import jax.numpy as jnp
from jax.experimental import pallas as pl
from jax.experimental.pallas import tpu as pltpu

S, D, H, DH, F = 2048, 512, 32, 16, 1792
G = 4
TQ = 512
KC = 128
TM = 256
NQ = S // TQ
NI = H * NQ
EPS = 1e-5
QSCALE = (DH ** -0.5) * 1.4426950408889634
f32, bf16 = jnp.float32, jnp.bfloat16

_NT = (((1,), (1,)), ((), ()))
_TN = (((0,), (0,)), ((), ()))


def _layernorm(x):
    mean = jnp.mean(x, axis=-1, keepdims=True)
    xc = x - mean
    var = jnp.mean(xc * xc, axis=-1, keepdims=True)
    return (xc * jax.lax.rsqrt(var + EPS)).astype(bf16)


def _mish(h):
    e = jnp.exp(-jnp.abs(h))
    sp = jnp.log1p(e) + jnp.maximum(h, 0.0)
    return h * jnp.tanh(sp)


def kernel(x_ref, wqkv_ref, wo_ref, w1_ref, b1_ref, w2_ref, o_ref,
           xs, wqT, wvT, q_scr, k_scr, v_scr, oT_scr, sA, sB):
    wqT[...] = wqkv_ref[:, 0:D].T
    wvT[...] = wqkv_ref[:, 2 * D:3 * D].T

    def qkv_block(r0, x):
        xn = _layernorm(x)
        kk = jnp.dot(xn, wqkv_ref[:, D:2 * D], preferred_element_type=f32).astype(bf16)
        qT = (jax.lax.dot_general(wqT[...], xn, _NT, preferred_element_type=f32) * QSCALE).astype(bf16)
        vT = jax.lax.dot_general(wvT[...], xn, _NT, preferred_element_type=f32).astype(bf16)
        for g in range(G):
            k_scr[g, pl.ds(r0, TM), :] = kk[:, g * 128:(g + 1) * 128]
            q_scr[g, :, pl.ds(r0, TM)] = qT[g * 128:(g + 1) * 128, :]
        v_scr[:, :, pl.ds(r0, TM)] = vT.reshape(H, DH, TM)

    def post_block(r0):
        oT = oT_scr[:, :, pl.ds(r0, TM)].reshape(D, TM)
        y = xs[pl.ds(r0, TM), :] + jax.lax.dot_general(oT, wo_ref[...], _TN, preferred_element_type=f32)
        yn = _layernorm(y)
        h = jnp.dot(yn, w1_ref[...], preferred_element_type=f32) + b1_ref[...].astype(f32)
        a = _mish(h).astype(bf16)
        return y + jnp.dot(a, w2_ref[...], preferred_element_type=f32)

    row = jax.lax.broadcasted_iota(jnp.int32, (128, TQ), 0) // DH

    def item(i):
        h = i // NQ
        q0 = pl.multiple_of((i % NQ) * TQ, TQ)
        return h, h // 8, h % 8, q0

    def both(i_new, s_new_ref, i_cur, s_cur_ref, m):
        if i_new is not None:
            _, g, j, q0n = item(i_new)
            qg = q_scr[g, :, pl.ds(q0n, TQ)]
            W = jnp.where(row == j, qg, jnp.zeros_like(qg))
            mx = jnp.full((8, TQ), -jnp.inf, f32)
        if i_cur is not None:
            h, _, _, q0 = item(i_cur)
            l = jnp.zeros((8, TQ), f32)
            acc = jnp.zeros((DH, TQ), f32)
        for c in range(S // KC):
            ks = slice(c * KC, (c + 1) * KC)
            if i_new is not None:
                s_new = jnp.dot(k_scr[g, ks, :], W, preferred_element_type=f32)
                s_new_ref[ks, :] = s_new
                mx = jnp.maximum(mx, jnp.max(s_new.reshape(KC // 8, 8, TQ), axis=0))
            if i_cur is not None:
                s = s_cur_ref[ks, :].reshape(KC // 8, 8, TQ)
                p = jnp.exp2(s - m[None])
                ps = [p[r] for r in range(KC // 8)]
                while len(ps) > 1:
                    ps = [ps[2 * t] + ps[2 * t + 1] for t in range(len(ps) // 2)]
                l = l + ps[0]
                pb = p.reshape(KC, TQ).astype(bf16)
                acc = acc + jnp.dot(v_scr[h, :, ks], pb, preferred_element_type=f32)
        if i_cur is not None:
            lsum = jnp.sum(l, axis=0, keepdims=True)
            oT_scr[h, :, pl.ds(q0, TQ)] = (acc / lsum).astype(bf16)
        if i_new is not None:
            return jnp.broadcast_to(jnp.max(mx, axis=0, keepdims=True), mx.shape)
        return m

    def attention():
        m0 = both(0, sA, None, None, None)

        def body(i, m):
            return jax.lax.cond(i % 2 == 0,
                                lambda: both(i + 1, sB, i, sA, m),
                                lambda: both(i + 1, sA, i, sB, m))
        m = jax.lax.fori_loop(0, NI - 1, body, m0)
        both(None, None, NI - 1, sB, m)

    def first_body(rb, _):
        r0 = pl.multiple_of(rb * TM, TM)
        x = x_ref[pl.ds(r0, TM), :].astype(f32)
        xs[pl.ds(r0, TM), :] = x
        qkv_block(r0, x)
        return 0
    jax.lax.fori_loop(0, S // TM, first_body, 0)

    def layer(li, _):
        attention()

        def dense_body(rb, _):
            r0 = pl.multiple_of(rb * TM, TM)
            x = post_block(r0)

            @pl.when(li == 0)
            def _():
                xs[pl.ds(r0, TM), :] = x
                qkv_block(r0, x)

            @pl.when(li == 1)
            def _():
                o_ref[pl.ds(r0, TM), :] = x.astype(o_ref.dtype)
            return 0
        jax.lax.fori_loop(0, S // TM, dense_body, 0)
        return 0
    jax.lax.fori_loop(0, 2, layer, 0)


@jax.jit
def pallas_interleave_layers__mha_block__dense_activation_mish__prompt_kernel(
    A_x, A_wqkv, A_wo, B_x, B_w1, B_b1, B_w2,
):
    del B_x
    x = A_x.reshape(S, D)
    b1 = B_b1.reshape(1, F)
    out = pl.pallas_call(
        kernel,
        out_shape=jax.ShapeDtypeStruct((S, D), A_x.dtype),
        scratch_shapes=[
            pltpu.VMEM((S, D), f32),
            pltpu.VMEM((D, D), bf16),
            pltpu.VMEM((D, D), bf16),
            pltpu.VMEM((G, 128, S), bf16),
            pltpu.VMEM((G, S, 128), bf16),
            pltpu.VMEM((H, DH, S), bf16),
            pltpu.VMEM((H, DH, S), bf16),
            pltpu.VMEM((S, TQ), f32),
            pltpu.VMEM((S, TQ), f32),
        ],
        compiler_params=pltpu.CompilerParams(vmem_limit_bytes=100 * 2**20),
    )(x, A_wqkv, A_wo, B_w1, b1, B_w2)
    return out.reshape(A_x.shape)
```

```python
import jax
import jax.numpy as jnp
from jax.experimental import pallas as pl
from jax.experimental.pallas import tpu as pltpu

S, D, H, DH, F = 2048, 512, 32, 16, 1792
TQ = 512
U = S // TQ
KC = 128
NC = S // KC
NQT = TQ // 128
TP = 512
NT = S // TP
SUB = ((0, 128), (128, 384))
HS = 16
VCH = (2, 6, 10, 14)
GS, LAG = 2, 2
VWORK = [(cv, half, n0) for cv in VCH for half in range(2) for n0 in range(0, NQT, GS)]
EPS = 1e-5
QSCALE = (DH ** -0.5) * 1.4426950408889634
f32, bf16, u32 = jnp.float32, jnp.bfloat16, jnp.uint32
_NT = (((1,), (1,)), ((), ()))


def _layernorm(x):
    mean = jnp.mean(x, axis=-1, keepdims=True)
    xc = x - mean
    var = jnp.mean(xc * xc, axis=-1, keepdims=True)
    return (xc * jax.lax.rsqrt(var + EPS)).astype(bf16)


def _mish(h):
    sp = jnp.log1p(jnp.exp(-jnp.abs(h))) + jnp.maximum(h, 0.0)
    return h * jnp.tanh(sp)


def _kernel(x_hbm, wqkv_hbm, wo_hbm, w1_hbm, b1_hbm, w2_hbm, o_hbm,
            x_ref, wqkv_ref, wo_ref, w1_ref, w2_ref, o_ref,
            xs, xn_scr, wqT, wvT, woT, q_scr, q32, k_scr, v_scr, oT_scr,
            sA, sB, kbA, kbB, mA, mB, accA, accB, lA, lB,
            b1_ref, sem_x, sem_w, sem_o):

    def x_copy(t):
        r = pl.multiple_of(t * TP, TP)
        return pltpu.make_async_copy(x_hbm.at[pl.ds(r, TP)], x_ref.at[pl.ds(r, TP)], sem_x.at[t])

    def o_copy(t):
        r = pl.multiple_of(t * TP, TP)
        return pltpu.make_async_copy(o_ref.at[pl.ds(r, TP)], o_hbm.at[pl.ds(r, TP)], sem_o.at[t])

    cq, ck, cv = [pltpu.make_async_copy(wqkv_hbm.at[:, n * D:(n + 1) * D], wqkv_ref.at[:, n * D:(n + 1) * D],
                                        sem_w.at[n]) for n in range(3)]
    w_copies = [pltpu.make_async_copy(src, dst, sem_w.at[3 + n]) for n, (src, dst) in enumerate(
        [(wo_hbm, wo_ref), (w1_hbm, w1_ref), (b1_hbm, b1_ref), (w2_hbm, w2_ref)])]

    def rows(t):
        return [(pl.multiple_of(t * TP + off, 128), n) for off, n in SUB]

    def ingest(t):
        x_copy(t).wait()
        for u, (r, n) in enumerate(rows(t)):
            x = x_ref[pl.ds(r, n), :].astype(f32)
            xs[pl.ds(r, n), :] = x
            if u == 0:
                xn_scr[pl.ds(r, n), :] = _layernorm(x)

    def out_proj(r, n):
        oT = oT_scr[HS:H, :, pl.ds(r, n)].reshape((H - HS) * DH, n)
        return xs[pl.ds(r, n), :] + jnp.dot(woT[:, HS * DH:], oT, preferred_element_type=f32).T

    def mlp_in(y):
        h = jnp.dot(_layernorm(y), w1_ref[...], preferred_element_type=f32)
        return _mish(h + b1_ref[...].astype(f32).reshape(1, F)).astype(bf16)

    def post(t):
        rs = rows(t)
        ys = [out_proj(r, n) for r, n in rs]
        acts = [mlp_in(y) for y in ys]
        xv = [y + jnp.dot(a, w2_ref[...], preferred_element_type=f32) for y, a in zip(ys, acts)]
        for (r, n), x in zip(rs, xv):
            xs[pl.ds(r, n), :] = x
            o_ref[pl.ds(r, n), :] = x.astype(o_ref.dtype)
        xn_scr[pl.ds(rs[0][0], rs[0][1]), :] = _layernorm(xv[0])

    def qkv(t):
        for u, (r, n) in enumerate(rows(t)):
            xn = xn_scr[pl.ds(r, n), :] if u == 0 else _layernorm(xs[pl.ds(r, n), :])
            kk = jnp.dot(xn, wqkv_ref[:, D:2 * D], preferred_element_type=f32).astype(bf16)
            for h in range(H):
                kg = pltpu.bitcast(kk[:, (h // 8) * 128:(h // 8 + 1) * 128], u32)
                if h % 8:
                    kg = pltpu.roll(kg, 128 - DH * (h % 8), 1)
                k_scr[h, pl.ds(pl.multiple_of(r // 2, 64), n // 2), :] = kg
            qT = (jax.lax.dot_general(wqT[...], xn, _NT, preferred_element_type=f32) * QSCALE).astype(bf16)
            q_scr[:, :, pl.ds(r, n)] = pltpu.bitcast(qT, u32).reshape(H, DH // 2, n)
            q32[:, :, pl.ds(r, n)] = qT.astype(f32).reshape(H, DH, n)
            vT = jax.lax.dot_general(wvT[...], xn, _NT, preferred_element_type=f32).astype(bf16)
            v_scr[:, :, pl.ds(r, n)] = pltpu.bitcast(vT, u32).reshape(H, DH // 2, n)

    def keys(h, k0, k1):
        return pltpu.bitcast(k_scr[h, k0 // 2:k1 // 2, :], bf16)

    def build_key_table(h, kb_ref):
        kt = jnp.concatenate([keys(h, c * KC, c * KC + 16) for c in VCH], axis=0).astype(f32)
        for d in range(DH):
            kb_ref[d] = jnp.broadcast_to(kt[:, d:d + 1], (16 * len(VCH), 128))

    def normalize(h, acc, l):
        for u in range(U):
            lsum = jnp.sum(l[u], axis=0, keepdims=True)
            oT_scr[h, :, u * TQ:(u + 1) * TQ] = (acc[u] / lsum).astype(bf16)

    def block(h_new, new, h_cur, cur, h_next, h_prev):
        split = h_new is not None and h_cur is not None
        mx, l, acc = [None] * U, [None] * U, [None] * U
        mxv = [[None] * NQT for _ in range(U)]
        ties = []
        if h_new is not None:
            zeros = jnp.zeros((64 - DH // 2, TQ), u32)
            Ws = [pltpu.bitcast(jnp.concatenate([q_scr[h_new, :, u * TQ:(u + 1) * TQ], zeros], axis=0), bf16)
                  for u in range(U)]
        if h_cur is not None:
            ms = [jnp.broadcast_to(jnp.max(cur["mx"][u], axis=0, keepdims=True), (8, TQ)) for u in range(U)]
        if h_prev is not None:
            normalize(h_prev, new["acc"], new["l"])

        def scores(u, c):
            k0, k1 = c * KC + (16 if split and c in VCH else 0), (c + 1) * KC
            s = jnp.dot(keys(h_new, k0, k1), Ws[u], preferred_element_type=f32)
            new["s"][k0:k1, u * TQ:(u + 1) * TQ] = s
            cm = jnp.max(s.reshape((k1 - k0) // 8, 8, TQ), axis=0)
            mx[u] = cm if c == 0 else jnp.maximum(mx[u], cm)
            touched = {}
            for cv, half, n0 in (VWORK[c * len(VWORK) // NC:(c + 1) * len(VWORK) // NC] if split else ()):
                r, row = 16 * VCH.index(cv) + 8 * half, cv * KC + 8 * half
                sv = {}
                for d in range(DH):
                    kv = new["kb"][d, r:r + 8, :]
                    for n in range(n0, n0 + GS):
                        q0 = u * TQ + n * 128
                        t = kv * jnp.broadcast_to(q32[h_new, d:d + 1, q0:q0 + 128], (8, 128))
                        sv[n] = t if d == 0 else sv[n] + t
                for n, v in sv.items():
                    q0 = u * TQ + n * 128
                    new["s"][row:row + 8, q0:q0 + 128] = v
                    mxv[u][n] = v if mxv[u][n] is None else jnp.maximum(mxv[u][n], v)
                    touched[n] = mxv[u][n]
            ties.append(touched)

        def softmax_pv(u, c, prev):
            ks = slice(c * KC, (c + 1) * KC)
            m = ms[u]
            if split and len(ties) > LAG:
                tiles = [m[:, n * 128:(n + 1) * 128] for n in range(NQT)]
                m = jnp.concatenate([x + 0.0 * ties[-LAG - 1][n] if n in ties[-LAG - 1] else x
                                     for n, x in enumerate(tiles)], axis=1)
            p = jnp.exp2(cur["s"][ks, u * TQ:(u + 1) * TQ].reshape(KC // 8, 8, TQ) - m[None])
            ps = [p[r] for r in range(KC // 8)]
            while len(ps) > 1:
                ps = [ps[2 * i] + ps[2 * i + 1] for i in range(len(ps) // 2)]
            l[u] = ps[0] if c == 0 else l[u] + ps[0]
            pv = jnp.dot(pltpu.bitcast(v_scr[h_cur, :, ks], bf16), p.reshape(KC, TQ).astype(bf16),
                         preferred_element_type=f32)
            acc[u] = pv if c == 0 else acc[u] + pv
            if h_new is None:
                r0, d0 = (2 * u + c // 8) * (TQ // 2), (c % 8) * 64
                oT = oT_scr[0:HS, :, r0:r0 + TQ // 2].reshape(HS * DH, TQ // 2)
                part = jnp.dot(woT[d0:d0 + 64, 0:HS * DH], oT, preferred_element_type=f32)
                if c % 2:
                    xs[r0:r0 + TQ // 2, d0 - 64:d0 + 64] += jnp.concatenate([prev, part], axis=0).T
                return part

        for u in range(U):
            prev = None
            for c in range(NC):
                if h_new is not None:
                    scores(u, c)
                if h_cur is not None:
                    prev = softmax_pv(u, c, prev)
        for u in range(U):
            if split:
                cur["acc"][u], cur["l"][u] = acc[u], l[u]
            if h_new is not None:
                new["mx"][u] = jnp.maximum(mx[u], jnp.concatenate(mxv[u], axis=1)) if split else mx[u]
        if h_new is None:
            normalize(h_cur, acc, l)
        if h_next is not None:
            build_key_table(h_next, (cur or B)["kb"])
        if h_cur is None:
            woT[...] = wo_ref[...].T

    A = dict(s=sA, kb=kbA, mx=mA, acc=accA, l=lA)
    B = dict(s=sB, kb=kbB, mx=mB, acc=accB, l=lB)

    def attention():
        accB[...] = jnp.zeros_like(accB)
        lB[...] = jnp.ones_like(lB)
        block(0, A, None, None, 1, None)

        def body(i, _):
            nxt, prev = jnp.minimum(i + 2, H - 1), jnp.maximum(i - 1, 0)
            jax.lax.cond((i & 1) == 0,
                         lambda: block(i + 1, B, i, A, nxt, prev),
                         lambda: block(i + 1, A, i, B, nxt, prev))
            return 0
        jax.lax.fori_loop(0, H - 1, body, 0)
        block(None, A, H - 1, B, None, H - 2)

    def phase(ph, _):
        def dense_step(t, _):
            @pl.when((ph == 0) & (t > 0))
            def _():
                ingest(t)

            @pl.when(ph > 0)
            def _():
                post(t)

            @pl.when(ph < 2)
            def _():
                qkv(t)

            @pl.when(ph == 2)
            def _():
                o_copy(t).start()
            return 0
        jax.lax.fori_loop(0, NT, dense_step, 0)

        @pl.when(ph == 0)
        def _():
            for cp in w_copies:
                cp.wait()

        @pl.when(ph < 2)
        def _():
            attention()
        return 0

    x_copy(0).start()
    for cp in (cq, cv, ck):
        cp.start()
    ingest(0)
    cq.wait()
    wqT[...] = wqkv_ref[:, 0:D].T
    cv.wait()
    wvT[...] = wqkv_ref[:, 2 * D:3 * D].T
    ck.wait()
    for t in range(1, NT):
        x_copy(t).start()
    for cp in w_copies:
        cp.start()
    jax.lax.fori_loop(0, 3, phase, 0)
    for t in range(NT):
        o_copy(t).wait()


@jax.jit
def pallas_interleave_layers__mha_block__dense_activation_mish__prompt_kernel(
    A_x, A_wqkv, A_wo, B_x, B_w1, B_b1, B_w2,
):
    del B_x
    out = pl.pallas_call(
        _kernel,
        out_shape=jax.ShapeDtypeStruct((S, D), A_x.dtype),
        in_specs=[pl.BlockSpec(memory_space=pl.ANY)] * 6,
        out_specs=pl.BlockSpec(memory_space=pl.ANY),
        scratch_shapes=[
            pltpu.VMEM((S, D), bf16),
            pltpu.VMEM((D, 3 * D), bf16),
            pltpu.VMEM((D, D), bf16),
            pltpu.VMEM((D, F), bf16),
            pltpu.VMEM((F, D), bf16),
            pltpu.VMEM((S, D), bf16),
            pltpu.VMEM((S, D), f32),
            pltpu.VMEM((S, D), bf16),
            pltpu.VMEM((D, D), bf16),
            pltpu.VMEM((D, D), bf16),
            pltpu.VMEM((D, D), bf16),
            pltpu.VMEM((H, DH // 2, S), u32),
            pltpu.VMEM((H, DH, S), f32),
            pltpu.VMEM((H, S // 2, 128), u32),
            pltpu.VMEM((H, DH // 2, S), u32),
            pltpu.VMEM((H, DH, S), bf16),
            pltpu.VMEM((S, S), f32),
            pltpu.VMEM((S, S), f32),
            pltpu.VMEM((DH, 16 * len(VCH), 128), f32),
            pltpu.VMEM((DH, 16 * len(VCH), 128), f32),
            pltpu.VMEM((U, 8, TQ), f32),
            pltpu.VMEM((U, 8, TQ), f32),
            pltpu.VMEM((U, DH, TQ), f32),
            pltpu.VMEM((U, DH, TQ), f32),
            pltpu.VMEM((U, 8, TQ), f32),
            pltpu.VMEM((U, 8, TQ), f32),
            pltpu.VMEM((F,), bf16),
            pltpu.SemaphoreType.DMA((NT,)),
            pltpu.SemaphoreType.DMA((7,)),
            pltpu.SemaphoreType.DMA((NT,)),
        ],
        compiler_params=pltpu.CompilerParams(vmem_limit_bytes=100 * 2**20),
    )(A_x.reshape(S, D), A_wqkv, A_wo, B_w1, B_b1, B_w2)
    return out.reshape(A_x.shape)
```

```python
import jax
import jax.numpy as jnp
from jax.experimental import pallas as pl
from jax.experimental.pallas import tpu as pltpu

S, D, H, DH, F = 2048, 512, 32, 16, 1792
TQ = 512
U = S // TQ
KC = 128
NC = S // KC
NQT = TQ // 128
TP = 512
NT = S // TP
SUB = ((0, 128), (128, 384))
HS = 16
VCH = (1, 3, 5, 7, 9, 11, 13, 15)
GS, LAG = 2, 2
VWORK = [(cv, half, n0) for cv in VCH for half in range(2) for n0 in range(0, NQT, GS)]
EPS = 1e-5
QSCALE = (DH ** -0.5) * 1.4426950408889634
f32, bf16, u32 = jnp.float32, jnp.bfloat16, jnp.uint32
_NT = (((1,), (1,)), ((), ()))


def _layernorm(x):
    mean = jnp.mean(x, axis=-1, keepdims=True)
    xc = x - mean
    var = jnp.mean(xc * xc, axis=-1, keepdims=True)
    return (xc * jax.lax.rsqrt(var + EPS)).astype(bf16)


def _mish(h):
    sp = jnp.log1p(jnp.exp(-jnp.abs(h))) + jnp.maximum(h, 0.0)
    return h * jnp.tanh(sp)


def _kernel(x_hbm, wqkv_hbm, wo_hbm, w1_hbm, b1_hbm, w2_hbm, o_hbm,
            x_ref, wqkv_ref, wo_ref, w1_ref, w2_ref, o_ref,
            xs, xn_scr, wqT, wvT, woT, q_scr, q32, k_scr, v_scr, oT_scr,
            sA, sB, kbA, kbB, mA, mB, accA, accB, lA, lB,
            b1_ref, sem_x, sem_w, sem_o):

    def x_copy(t):
        r = pl.multiple_of(t * TP, TP)
        return pltpu.make_async_copy(x_hbm.at[pl.ds(r, TP)], x_ref.at[pl.ds(r, TP)], sem_x.at[t])

    def o_copy(t):
        r = pl.multiple_of(t * TP, TP)
        return pltpu.make_async_copy(o_ref.at[pl.ds(r, TP)], o_hbm.at[pl.ds(r, TP)], sem_o.at[t])

    cq, ck, cv = [pltpu.make_async_copy(wqkv_hbm.at[:, n * D:(n + 1) * D], wqkv_ref.at[:, n * D:(n + 1) * D],
                                        sem_w.at[n]) for n in range(3)]
    w_copies = [pltpu.make_async_copy(src, dst, sem_w.at[3 + n]) for n, (src, dst) in enumerate(
        [(wo_hbm, wo_ref), (w1_hbm, w1_ref), (b1_hbm, b1_ref), (w2_hbm, w2_ref)])]

    def rows(t):
        return [(pl.multiple_of(t * TP + off, 128), n) for off, n in SUB]

    def ingest(t):
        x_copy(t).wait()
        for u, (r, n) in enumerate(rows(t)):
            x = x_ref[pl.ds(r, n), :].astype(f32)
            xs[pl.ds(r, n), :] = x
            if u == 0:
                xn_scr[pl.ds(r, n), :] = _layernorm(x)

    def out_proj(r, n):
        oT = oT_scr[HS:H, :, pl.ds(r, n)].reshape((H - HS) * DH, n)
        return xs[pl.ds(r, n), :] + jnp.dot(woT[:, HS * DH:], oT, preferred_element_type=f32).T

    def mlp_in(y):
        h = jnp.dot(_layernorm(y), w1_ref[...], preferred_element_type=f32)
        return _mish(h + b1_ref[...].astype(f32).reshape(1, F)).astype(bf16)

    def post(t):
        rs = rows(t)
        ys = [out_proj(r, n) for r, n in rs]
        acts = [mlp_in(y) for y in ys]
        xv = [y + jnp.dot(a, w2_ref[...], preferred_element_type=f32) for y, a in zip(ys, acts)]
        for (r, n), x in zip(rs, xv):
            xs[pl.ds(r, n), :] = x
            o_ref[pl.ds(r, n), :] = x.astype(o_ref.dtype)
        xn_scr[pl.ds(rs[0][0], rs[0][1]), :] = _layernorm(xv[0])

    def qkv(t):
        for u, (r, n) in enumerate(rows(t)):
            xn = xn_scr[pl.ds(r, n), :] if u == 0 else _layernorm(xs[pl.ds(r, n), :])
            kk = jnp.dot(xn, wqkv_ref[:, D:2 * D], preferred_element_type=f32).astype(bf16)
            for h in range(H):
                kg = pltpu.bitcast(kk[:, (h // 8) * 128:(h // 8 + 1) * 128], u32)
                if h % 8:
                    kg = pltpu.roll(kg, 128 - DH * (h % 8), 1)
                k_scr[h, pl.ds(pl.multiple_of(r // 2, 64), n // 2), :] = kg
            qT = (jax.lax.dot_general(wqT[...], xn, _NT, preferred_element_type=f32) * QSCALE).astype(bf16)
            q_scr[:, :, pl.ds(r, n)] = pltpu.bitcast(qT, u32).reshape(H, DH // 2, n)
            q32[:, :, pl.ds(r, n)] = qT.astype(f32).reshape(H, DH, n)
            vT = jax.lax.dot_general(wvT[...], xn, _NT, preferred_element_type=f32).astype(bf16)
            v_scr[:, :, pl.ds(r, n)] = pltpu.bitcast(vT, u32).reshape(H, DH // 2, n)

    def keys(h, k0, k1):
        return pltpu.bitcast(k_scr[h, k0 // 2:k1 // 2, :], bf16)

    def build_key_table(h, kb_ref):
        kt = jnp.concatenate([keys(h, c * KC, c * KC + 16) for c in VCH], axis=0).astype(f32)
        for d in range(DH):
            kb_ref[d] = jnp.broadcast_to(kt[:, d:d + 1], (16 * len(VCH), 128))

    def normalize(h, acc, l):
        for u in range(U):
            lsum = jnp.sum(l[u], axis=0, keepdims=True)
            oT_scr[h, :, u * TQ:(u + 1) * TQ] = (acc[u] / lsum).astype(bf16)

    def block(h_new, new, h_cur, cur, h_next, h_prev):
        split = h_new is not None and h_cur is not None
        mx, l, acc = [None] * U, [None] * U, [None] * U
        mxv = [[None] * NQT for _ in range(U)]
        ties = []
        if h_new is not None:
            zeros = jnp.zeros((64 - DH // 2, TQ), u32)
            Ws = [jnp.concatenate([q_scr[h_new, :, u * TQ:(u + 1) * TQ], zeros], axis=0) for u in range(U)]
        if h_cur is not None:
            ms = [jnp.broadcast_to(jnp.max(cur["mx"][u], axis=0, keepdims=True), (8, TQ)) for u in range(U)]
        if h_prev is not None:
            normalize(h_prev, new["acc"], new["l"])

        def scores(u, c):
            k0, k1 = c * KC + (16 if split and c in VCH else 0), (c + 1) * KC
            s = jnp.dot(keys(h_new, k0, k1), pltpu.bitcast(Ws[u], bf16), preferred_element_type=f32)
            new["s"][k0:k1, u * TQ:(u + 1) * TQ] = s
            cm = jnp.max(s.reshape((k1 - k0) // 8, 8, TQ), axis=0)
            mx[u] = cm if c == 0 else jnp.maximum(mx[u], cm)
            touched = {}
            for cv, half, n0 in (VWORK[c * len(VWORK) // NC:(c + 1) * len(VWORK) // NC] if split else ()):
                r, row = 16 * VCH.index(cv) + 8 * half, cv * KC + 8 * half
                sv = {}
                for d in range(DH):
                    kv = new["kb"][d, r:r + 8, :]
                    for n in range(n0, n0 + GS):
                        q0 = u * TQ + n * 128
                        t = kv * jnp.broadcast_to(q32[h_new, d:d + 1, q0:q0 + 128], (8, 128))
                        sv[n] = t if d == 0 else sv[n] + t
                for n, v in sv.items():
                    q0 = u * TQ + n * 128
                    new["s"][row:row + 8, q0:q0 + 128] = v
                    mxv[u][n] = v if mxv[u][n] is None else jnp.maximum(mxv[u][n], v)
                    touched[n] = mxv[u][n]
            ties.append(touched)

        def softmax_pv(u, c, prev):
            ks = slice(c * KC, (c + 1) * KC)
            m = ms[u]
            if split and len(ties) > LAG:
                tiles = [m[:, n * 128:(n + 1) * 128] for n in range(NQT)]
                m = jnp.concatenate([x + 0.0 * ties[-LAG - 1][n] if n in ties[-LAG - 1] else x
                                     for n, x in enumerate(tiles)], axis=1)
            p = jnp.exp2(cur["s"][ks, u * TQ:(u + 1) * TQ].reshape(KC // 8, 8, TQ) - m[None])
            ps = [p[r] for r in range(KC // 8)]
            while len(ps) > 1:
                ps = [ps[2 * i] + ps[2 * i + 1] for i in range(len(ps) // 2)]
            l[u] = ps[0] if c == 0 else l[u] + ps[0]
            pv = jnp.dot(pltpu.bitcast(v_scr[h_cur, :, ks], bf16), p.reshape(KC, TQ).astype(bf16),
                         preferred_element_type=f32)
            acc[u] = pv if c == 0 else acc[u] + pv
            if h_new is None:
                r0, d0 = (2 * u + c // 8) * (TQ // 2), (c % 8) * 64
                oT = oT_scr[0:HS, :, r0:r0 + TQ // 2].reshape(HS * DH, TQ // 2)
                part = jnp.dot(woT[d0:d0 + 64, 0:HS * DH], oT, preferred_element_type=f32)
                if c % 2:
                    xs[r0:r0 + TQ // 2, d0 - 64:d0 + 64] += jnp.concatenate([prev, part], axis=0).T
                return part

        for u in range(U):
            prev = None
            for c in range(NC):
                if h_new is not None:
                    scores(u, c)
                if h_cur is not None:
                    prev = softmax_pv(u, c, prev)
        for u in range(U):
            if split:
                cur["acc"][u], cur["l"][u] = acc[u], l[u]
            if h_new is not None:
                new["mx"][u] = jnp.maximum(mx[u], jnp.concatenate(mxv[u], axis=1)) if split else mx[u]
        if h_new is None:
            normalize(h_cur, acc, l)
        if h_next is not None:
            build_key_table(h_next, (cur or B)["kb"])
        if h_cur is None:
            woT[...] = wo_ref[...].T

    A = dict(s=sA, kb=kbA, mx=mA, acc=accA, l=lA)
    B = dict(s=sB, kb=kbB, mx=mB, acc=accB, l=lB)

    def attention():
        accB[...] = jnp.zeros_like(accB)
        lB[...] = jnp.ones_like(lB)
        block(0, A, None, None, 1, None)

        def body(i, _):
            nxt, prev = jnp.minimum(i + 2, H - 1), jnp.maximum(i - 1, 0)
            jax.lax.cond((i & 1) == 0,
                         lambda: block(i + 1, B, i, A, nxt, prev),
                         lambda: block(i + 1, A, i, B, nxt, prev))
            return 0
        jax.lax.fori_loop(0, H - 1, body, 0)
        block(None, A, H - 1, B, None, H - 2)

    def phase(ph, _):
        def dense_step(t, _):
            @pl.when((ph == 0) & (t > 0))
            def _():
                ingest(t)

            @pl.when(ph > 0)
            def _():
                post(t)

            @pl.when(ph < 2)
            def _():
                qkv(t)

            @pl.when(ph == 2)
            def _():
                o_copy(t).start()
            return 0
        jax.lax.fori_loop(0, NT, dense_step, 0)

        @pl.when(ph == 0)
        def _():
            for cp in w_copies:
                cp.wait()

        @pl.when(ph < 2)
        def _():
            attention()
        return 0

    x_copy(0).start()
    for cp in (cq, cv, ck):
        cp.start()
    ingest(0)
    cq.wait()
    wqT[...] = wqkv_ref[:, 0:D].T
    cv.wait()
    wvT[...] = wqkv_ref[:, 2 * D:3 * D].T
    ck.wait()
    for t in range(1, NT):
        x_copy(t).start()
    for cp in w_copies:
        cp.start()
    jax.lax.fori_loop(0, 3, phase, 0)
    for t in range(NT):
        o_copy(t).wait()


@jax.jit
def pallas_interleave_layers__mha_block__dense_activation_mish__prompt_kernel(
    A_x, A_wqkv, A_wo, B_x, B_w1, B_b1, B_w2,
):
    del B_x
    out = pl.pallas_call(
        _kernel,
        out_shape=jax.ShapeDtypeStruct((S, D), A_x.dtype),
        in_specs=[pl.BlockSpec(memory_space=pl.ANY)] * 6,
        out_specs=pl.BlockSpec(memory_space=pl.ANY),
        scratch_shapes=[
            pltpu.VMEM((S, D), bf16),
            pltpu.VMEM((D, 3 * D), bf16),
            pltpu.VMEM((D, D), bf16),
            pltpu.VMEM((D, F), bf16),
            pltpu.VMEM((F, D), bf16),
            pltpu.VMEM((S, D), bf16),
            pltpu.VMEM((S, D), f32),
            pltpu.VMEM((S, D), bf16),
            pltpu.VMEM((D, D), bf16),
            pltpu.VMEM((D, D), bf16),
            pltpu.VMEM((D, D), bf16),
            pltpu.VMEM((H, DH // 2, S), u32),
            pltpu.VMEM((H, DH, S), f32),
            pltpu.VMEM((H, S // 2, 128), u32),
            pltpu.VMEM((H, DH // 2, S), u32),
            pltpu.VMEM((H, DH, S), bf16),
            pltpu.VMEM((S, S), f32),
            pltpu.VMEM((S, S), f32),
            pltpu.VMEM((DH, 16 * len(VCH), 128), f32),
            pltpu.VMEM((DH, 16 * len(VCH), 128), f32),
            pltpu.VMEM((U, 8, TQ), f32),
            pltpu.VMEM((U, 8, TQ), f32),
            pltpu.VMEM((U, DH, TQ), f32),
            pltpu.VMEM((U, DH, TQ), f32),
            pltpu.VMEM((U, 8, TQ), f32),
            pltpu.VMEM((U, 8, TQ), f32),
            pltpu.VMEM((F,), bf16),
            pltpu.SemaphoreType.DMA((NT,)),
            pltpu.SemaphoreType.DMA((7,)),
            pltpu.SemaphoreType.DMA((NT,)),
        ],
        compiler_params=pltpu.CompilerParams(vmem_limit_bytes=100 * 2**20),
    )(A_x.reshape(S, D), A_wqkv, A_wo, B_w1, B_b1, B_w2)
    return out.reshape(A_x.shape)
```
